```python
import jax
import jax.numpy as jnp

def _softmax(x, axis=-1):
    return jax.nn.softmax(x, axis=axis)
def _gelu(x):
    return jax.nn.gelu(x, approximate=True)
def _silu(x):
    return jax.nn.silu(x)
def _sigmoid(x):
    return jax.nn.sigmoid(x)
def _layernorm(x, axis=-1, eps=1e-5):
    m = jnp.mean(x, axis=axis, keepdims=True)
    v = jnp.var(x, axis=axis, keepdims=True)
    return (x - m) / jnp.sqrt(v + eps)
def _scatter_add(tgt, idx, src, axis=0):
    return tgt.at[idx].add(src)
def _segment_sum(src, seg, n):
    return jax.ops.segment_sum(src, seg, n)
class _Rng:
    def __init__(self, key):
        self._k = key
    def _next(self):
        self._k, sub = jax.random.split(self._k)
        return sub
    def normal(self, shape):
        return jax.random.normal(self._next(), shape, dtype=jnp.bfloat16)
    def randint(self, lo, hi, shape):
        return jax.random.randint(self._next(), shape, lo, hi, dtype=jnp.int32)
    def uniform(self, shape, lo=0.0, hi=1.0):
        return jax.random.uniform(self._next(), shape, jnp.bfloat16, lo, hi)
    def permutation(self, n):
        return jax.random.permutation(self._next(), n)


kernel_name = 'recurrent_scan__sliding_block_cached__dense_activation_gelu__decode'

def setup_inputs():
    _rng = _Rng(jax.random.key(int.from_bytes(__import__("os").urandom(4), "little")))
    _w = (lambda a: (lambda t: t.astype(jnp.bfloat16) if jnp.issubdtype(t.dtype, jnp.floating) else t)(jnp.asarray(a)))
    def _A_setup():
        B, Sq, D = 2, 1, 576
        Hq, Hkv, Sk, Dh = 32, 16, 32768, 128
        assert Hq % Hkv == 0, (Hq, Hkv)
        return {
            "x": _w((lambda *s: _rng.normal(s) * 0.05)(B, Sq, D)),
            "k_cache": _w((lambda *s: _rng.normal(s) * 0.05)(B, Hkv, Sk, Dh)),
            "v_cache": _w((lambda *s: _rng.normal(s) * 0.05)(B, Hkv, Sk, Dh)),
            "wq": _w((lambda *s: _rng.normal(s) * 0.05)(D, Hq * Dh) * (D ** -0.5)),
            "wo": _w((lambda *s: _rng.normal(s) * 0.05)(Hq * Dh, D) * ((Hq * Dh) ** -0.5)),
        }
    _A_in = _A_setup()

    def _B_setup():
        B, S, D, F = 2, 1, 576, 4608
        return {
            "x": _w((lambda *s: _rng.normal(s) * 0.05)(B, S, D)),
            "w1": _w((lambda *s: _rng.normal(s) * 0.05)(D, F) * (D ** -0.5)),
            "b1": _w((lambda *s: _rng.normal(s) * 0.05)(F) * 0.01),
            "w2": _w((lambda *s: _rng.normal(s) * 0.05)(F, D) * (F ** -0.5)),
            "b2": _w((lambda *s: _rng.normal(s) * 0.05)(D) * 0.01),
        }
    _B_in = _B_setup()

    return {
        "A_x": _A_in["x"],
        "A_k_cache": _A_in["k_cache"],
        "A_v_cache": _A_in["v_cache"],
        "A_wq": _A_in["wq"],
        "A_wo": _A_in["wo"],
        "B_x": _B_in["x"],
        "B_w1": _B_in["w1"],
        "B_b1": _B_in["b1"],
        "B_w2": _B_in["w2"],
        "B_b2": _B_in["b2"],
    }

def reference(A_x, A_k_cache, A_v_cache, A_wq, A_wo, B_x, B_w1, B_b1, B_w2, B_b2):
    def _A_ref(x, k_cache, v_cache, wq, wo):
        B, Sq, D = x.shape
        Hq, Dh = 32, 128
        Hkv, Sk = k_cache.shape[1], k_cache.shape[2]
        W = min(4096, max(256, Sk // 4))
        rep = Hq // Hkv
        q = (lambda x, *d: x.transpose(*d))((x @ wq).reshape(B, Sq, Hq, Dh), 0, 2, 1, 3)
        k = jnp.repeat(k_cache[:, :, Sk - W:, :], rep, axis=1)
        v = jnp.repeat(v_cache[:, :, Sk - W:, :], rep, axis=1)
        scores = jnp.einsum("bhqd,bhkd->bhqk", q, k) * (Dh ** -0.5)
        p = _softmax(scores, axis=-1)
        o = jnp.einsum("bhqk,bhkd->bhqd", p, v)
        return (lambda x, *d: x.transpose(*d))(o, 0, 2, 1, 3).reshape(B, Sq, Hq * Dh) @ wo

    def _B_ref(x, w1, b1, w2, b2):
        h = jnp.einsum("bsd,df->bsf", x, w1) + b1
        h = _gelu(h)
        return jnp.einsum("bsf,fd->bsd", h, w2) + b2

    x = A_x
    xn = _layernorm(x, axis=-1)
    s = _A_ref(xn, A_k_cache, A_v_cache, A_wq, A_wo)
    g = _silu(_B_ref(xn, B_w1, B_b1, B_w2, B_b2))
    return x + s * g
```

```python
import itertools
import jax, jax.numpy as jnp
from jax import lax
from jax.experimental import pallas as pl
from jax.experimental.pallas import tpu as pltpu
bf = jnp.bfloat16
f32 = jnp.float32
HBM = pltpu.HBM
D, HKV, SK, DH, F, W = 576, 16, 32768, 128, 4608, 4096
NT = (((1,), (1,)), ((), ()))
CB = 512

def make(gr=128, dr=64, L=5, prio=lambda i: (i//2)%2, interleave=True, compute=True, wr=16, worder=None):
    worder = worder or list(range(0, D, wr))
    NG = W // gr
    NQ, N1 = 4096 // CB, F // CB
    kinds = [('q', NQ), ('1', N1), ('k', 2*NG), ('v', 2*NG), ('2', N1), ('o', NQ)]
    seq = [(k, i) for k, n in kinds for i in range(n)]
    steps = [(seq[t], seq[t+L] if t+L < len(seq) else None, t) for t in range(len(seq))]
    runs = [list(g) for _, g in itertools.groupby(steps, key=lambda s: (s[0][0], s[1][0] if s[1] else None))]

    def kern(x_h, k_h, v_h, wq_h, wo_h, w1_h, b1_h, w2_h, b2_h, o_ref,
             kb, vb, wqb, wob, w1b, w2b, xb, b1b, b2b, yq, y1, qs, sc, mx, acc, ls, sems, ssem):
        wsrc = {'q': (wq_h, wqb), '1': (w1_h, w1b), '2': (w2_h, w2b), 'o': (wo_h, wob)}
        def copies(kind, i, slot):
            if kind in wsrc:
                s, d = wsrc[kind]
                c0 = i * CB if isinstance(i, int) else pl.multiple_of(i * CB, CB)
                return [pltpu.make_async_copy(s.at[pl.ds(r, wr), pl.ds(c0, CB)], d.at[i, pl.ds(r, wr)], sems.at[slot])
                        for r in worder]
            s, d = (k_h, kb) if kind == 'k' else (v_h, vb)
            p = i // NG; r0 = (i % NG) * gr
            if not isinstance(r0, int): r0 = pl.multiple_of(r0, gr)
            return [pltpu.make_async_copy(s.at[j % 2, p * 8 + j // 2, pl.ds(SK - W + r0 + r, dr)], d.at[i, j, pl.ds(r, dr)], sems.at[slot])
                    for r in range(0, gr, dr) for j in range(HKV)]
        def wait_group(kind, i, slot):
            d = wsrc[kind][1] if kind in wsrc else (kb if kind == 'k' else vb)
            pltpu.make_async_copy(d.at[i], d.at[i], sems.at[slot]).wait()

        small = [pltpu.make_async_copy(x_h, xb, ssem), pltpu.make_async_copy(b1_h, b1b, ssem),
                 pltpu.make_async_copy(b2_h, b2b, ssem)]
        for t in range(L):
            for j, c in enumerate(copies(*seq[t], t % L)): c.start(priority=prio(j))
            if t == 0:
                for s in small: s.start()
        mx[...] = jnp.full(mx.shape, -jnp.inf, f32)
        acc[...] = jnp.zeros(acc.shape, f32)
        ls[...] = jnp.zeros(ls.shape, f32)
        for s in small: s.wait()

        row = lax.broadcasted_iota(jnp.int32, (8, D), 0)
        x0 = xb[0:1, :].astype(f32); x1 = xb[1:2, :].astype(f32)
        x8 = jnp.where(row % 2 == 0, x0, x1)
        m = jnp.mean(x8, axis=-1, keepdims=True)
        xc = x8 - m
        var = jnp.mean(xc * xc, axis=-1, keepdims=True)
        xn = (xc / jnp.sqrt(var + 1e-5)).astype(bf)
        scale = DH ** -0.5

        def pieces(kind, i, carry):
            if kind in ('q', '1'):
                src = wsrc[kind][1]; dst = yq if kind == 'q' else y1
                def mk(n):
                    def f(c):
                        dst[i, :, n*128:(n+1)*128] = jnp.dot(xn, src[i, :, n*128:(n+1)*128], preferred_element_type=f32)
                        return c
                    return f
                return [mk(n) for n in range(CB // 128)]
            if kind in ('2', 'o'):
                src = wsrc[kind][1]; lhs = y1 if kind == '2' else yq
                def mk(n):
                    def f(c):
                        return c + lax.dot_general(lhs[i, :, n*128:(n+1)*128].astype(bf), src[i, :, n*128:(n+1)*128], NT, preferred_element_type=f32)
                    return f
                return [mk(n) for n in range(CB // 128)]
            b = i // NG
            if kind == 'k':
                def mk(h):
                    def f(c):
                        s = lax.dot_general(qs[b * 8 + h // 2].astype(bf), kb[i, h], NT, preferred_element_type=f32) * scale
                        sc[i, h] = s
                        mm = mx[b, h]
                        for u in range(gr // 128): mm = jnp.maximum(mm, s[:, u*128:(u+1)*128])
                        mx[b, h] = mm
                        return c
                    return f
                return [mk(h) for h in range(HKV)]
            def mk(h):
                def f(c):
                    mm = mx[b, h]
                    s = sc[i, h]
                    ps = [jnp.exp(s[:, u*128:(u+1)*128] - mm) for u in range(gr // 128)]
                    ll = ls[b, h]
                    for p in ps: ll = ll + p
                    ls[b, h] = ll
                    p = ps[0] if len(ps) == 1 else jnp.concatenate(ps, axis=1)
                    acc[b, h] += jnp.dot(p.astype(bf), vb[i, h], preferred_element_type=f32)
                    return c
                return f
            return [mk(h) for h in range(HKV)]

        def step(ck, ci, ik, ii, slot, carry):
            wait_group(ck, ci, slot)
            cps = copies(ik, ii, slot) if ik else []
            pcs = pieces(ck, ci, carry) if (compute or ck not in 'kv') else []
            if not interleave or not pcs:
                for j, c in enumerate(cps): c.start(priority=prio(j))
                for p in pcs: carry = p(carry)
                return carry
            n = len(pcs); j = 0
            for u, p in enumerate(pcs):
                hi = (len(cps) * (u + 1)) // n
                while j < hi:
                    cps[j].start(priority=prio(j)); j += 1
                carry = p(carry)
            return carry

        r128 = lax.broadcasted_iota(jnp.int32, (8, DH), 0)
        carry = 0
        g = None
        prev = None
        for run in runs:
            (ck, c0), iss, t0 = run[0][0], run[0][1], run[0][2]
            if ck != prev:
                if prev == 'q':
                    for h in range(HKV):
                        o_ = (h % 2) * 256
                        qs[h] = jnp.where(r128 % 4 < 2, yq[h // 2, :, o_:o_+128], yq[h // 2, :, o_+128:o_+256])
                if prev == '1':
                    b1v = b1b[...].astype(f32).reshape(1, F)
                    for c in range(N1):
                        y1[c] = jax.nn.gelu(y1[c] + b1v[:, c*CB:(c+1)*CB], approximate=True)
                if prev == 'k':
                    for b in range(2):
                        for h in range(HKV):
                            mx[b, h] = jnp.broadcast_to(jnp.max(mx[b, h], axis=-1, keepdims=True), (8, DH))
                if prev == 'v':
                    for h in range(HKV):
                        oo = [acc[h // 8, (h % 8) * 2 + b] / jnp.sum(ls[h // 8, (h % 8) * 2 + b], axis=-1, keepdims=True) for b in range(2)]
                        c_ = jnp.where(r128 % 2 == 0, oo[0], oo[1])
                        o_ = (h % 2) * 256
                        yq[h // 2, :, o_:o_+128] = jnp.where(r128 % 4 < 2, c_, 0.0)
                        yq[h // 2, :, o_+128:o_+256] = jnp.where(r128 % 4 >= 2, c_, 0.0)
                if prev == '2':
                    g = carry + b2b[...].astype(f32).reshape(1, D)
                    g = g * jax.nn.sigmoid(g)
                if ck in '2o': carry = jnp.zeros((8, D), f32)
                prev = ck
            ik, i0 = iss if iss else (None, None)
            n = len(run)
            if n == 1 or ik is None:
                for u in range(n):
                    carry = step(ck, c0 + u, ik, (i0 + u) if ik else None, (t0 + u) % L, carry)
            else:
                def body(u, c, ck=ck, c0=c0, ik=ik, i0=i0, t0=t0):
                    return step(ck, c0 + u, ik, i0 + u, lax.rem(t0 + u, L), c)
                carry = lax.fori_loop(0, n, body, carry)
        s8 = carry + pltpu.roll(carry, 6, 0)
        res = x8 + s8 * g
        o_ref[...] = res[0:2].astype(bf)

    def f(x, k, v, wq, wo, bx, w1, b1, w2, b2):
        out = pl.pallas_call(kern, out_shape=jax.ShapeDtypeStruct((2, D), bf),
            in_specs=[pl.BlockSpec(memory_space=HBM)]*9,
            scratch_shapes=[pltpu.VMEM((2*NG,HKV,gr,DH),bf), pltpu.VMEM((2*NG,HKV,gr,DH),bf),
                pltpu.VMEM((NQ,D,CB),bf), pltpu.VMEM((NQ,D,CB),bf), pltpu.VMEM((N1,D,CB),bf), pltpu.VMEM((N1,D,CB),bf),
                pltpu.VMEM((2,D),bf), pltpu.VMEM((F,),bf), pltpu.VMEM((D,),bf),
                pltpu.VMEM((NQ,8,CB),f32), pltpu.VMEM((N1,8,CB),f32), pltpu.VMEM((HKV,8,DH),f32),
                pltpu.VMEM((2*NG,HKV,8,gr),f32),
                pltpu.VMEM((2,HKV,8,DH),f32), pltpu.VMEM((2,HKV,8,DH),f32), pltpu.VMEM((2,HKV,8,DH),f32),
                pltpu.SemaphoreType.DMA((L,)), pltpu.SemaphoreType.DMA(())],
            compiler_params=pltpu.CompilerParams(vmem_limit_bytes=110*2**20),
            )(x.reshape(2, D), k, v, wq, wo.T, w1, b1, w2.T, b2)
        return out.reshape(2, 1, D)
    return f


_impl = make()

@jax.jit
def pallas_recurrent_scan__sliding_block_cached__dense_activation_gelu__decode_kernel(
        A_x, A_k_cache, A_v_cache, A_wq, A_wo, B_x, B_w1, B_b1, B_w2, B_b2):
    return _impl(A_x, A_k_cache, A_v_cache, A_wq, A_wo, B_x, B_w1, B_b1, B_w2, B_b2)
```

```python
import itertools

import jax
import jax.numpy as jnp
from jax import lax
import jax.experimental.pallas as pl
import jax.experimental.pallas.tpu as pltpu

BF16 = jnp.bfloat16
F32 = jnp.float32
NT = (((1,), (1,)), ((), ()))

DH = 128
CB = 512
GR = 128
DR = 64
NS = 8
NC = 4
LOOKAHEAD = 4


def _aligned(x, m):
    return x if isinstance(x, int) else pl.multiple_of(x, m)


def _make_kernel(D, HKV, SK, W, FQ, FF):
    NG = W // GR
    NP = HKV // 8
    NQ, NF = FQ // CB, FF // CB
    SR = D // NS
    NW = SR // 8
    assert NQ <= NW and NF == NW and NF <= NP * NG

    seq = [(kind, i)
           for kind, n in (("wq", NW), ("w1", NW), ("w2", NW),
                           ("k", NP * NG), ("v", NP * NG), ("wo", NQ))
           for i in range(n)]

    def math_for(kind, i):
        if kind == "wq":
            return ()
        if kind == "w1":
            return ("q",) if i < NQ else ()
        if kind == "w2":
            return ("h",)
        if kind == "k" and i < NF:
            return ("g", "k")
        return (kind,)

    steps = [(seq[t], seq[t + LOOKAHEAD] if t + LOOKAHEAD < len(seq) else (None, None), t)
             for t in range(len(seq))]
    runs = [list(g) for _, g in itertools.groupby(
        steps, key=lambda s: (s[0][0], math_for(*s[0]), s[1][0]))]

    def kernel(x_h, k_h, v_h, wq_h, wo_h, w1_h, b1_h, w2_h, b2_h, o_ref,
               kb, vb, wqb, wob, w1b, w2b, xb, b1b, b2b,
               qs, hid, att, sc, mx, acc, den, sems, small_sems):
        rowmajor = {"wq": (wq_h, wqb), "w1": (w1_h, w1b), "w2": (w2_h, w2b)}

        def copies(kind, i, slot):
            sem = sems.at[slot]
            if kind in rowmajor:
                src, dst = rowmajor[kind]
                nc = src.shape[1] // NC
                out = []
                for u in range(NC):
                    for j in range(NS):
                        rows = pl.ds(_aligned(j * SR + i * 8, 8), 8)
                        cols = pl.ds(u * nc, nc)
                        out.append(pltpu.make_async_copy(
                            src.at[rows, cols], dst.at[rows, cols], sem))
                return out
            if kind == "wo":
                cols = pl.ds(_aligned(i * CB, CB), CB)
                return [pltpu.make_async_copy(
                            wo_h.at[pl.ds(r, 16), cols], wob.at[i, pl.ds(r, 16)], sem)
                        for r in range(0, D, 16)]
            src, dst = (k_h, kb) if kind == "k" else (v_h, vb)
            phase = i // NG
            r0 = _aligned((i % NG) * GR, GR)
            return [pltpu.make_async_copy(
                        src.at[j % 2, phase * 8 + j // 2, pl.ds(SK - W + r0 + r, DR)],
                        dst.at[i, j, pl.ds(r, DR)], sem)
                    for r in range(0, GR, DR) for j in range(16)]

        def start(cps, lo, hi):
            for j in range(lo, hi):
                cps[j].start(priority=(j // 2) % 2)

        small = [pltpu.make_async_copy(s, d, small_sems.at[n])
                 for n, (s, d) in enumerate(((x_h, xb), (b1_h, b1b), (b2_h, b2b)))]
        for t in range(LOOKAHEAD):
            cps = copies(*seq[t], t)
            start(cps, 0, len(cps))
            if t == 0:
                for c in small:
                    c.start()
        mx[...] = jnp.full(mx.shape, -jnp.inf, F32)
        acc[...] = jnp.zeros(acc.shape, F32)
        den[...] = jnp.zeros(den.shape, F32)
        for c in small:
            c.wait()

        row = lax.broadcasted_iota(jnp.int32, (8, D), 0)
        x8 = jnp.where(row % 2 == 0, xb[0:1, :].astype(F32), xb[1:2, :].astype(F32))
        xc = x8 - jnp.mean(x8, axis=-1, keepdims=True)
        var = jnp.mean(xc * xc, axis=-1, keepdims=True)
        xn = (xc / jnp.sqrt(var + 1e-5)).astype(BF16)
        b1 = b1b[...].astype(F32).reshape(1, FF)
        for c in range(NF):
            hid[c] = jnp.broadcast_to(b1[:, c * CB:(c + 1) * CB], (8, CB))
        first_head = lax.broadcasted_iota(jnp.int32, (8, DH), 0) % 4 < 2
        first_batch = lax.broadcasted_iota(jnp.int32, (8, DH), 0) % 2 == 0

        def cols128(i, n, width=128):
            return pl.ds(_aligned(i * CB + n * width, 128), width)

        def q_piece(i, u, c):
            y = jnp.dot(xn, wqb[:, cols128(i, u, 256)], preferred_element_type=F32)
            qs[2 * i + u] = jnp.where(first_head, y[:, :128], y[:, 128:])
            return c

        def h_piece(i, n, c):
            sl = slice(n * 128, (n + 1) * 128)
            y = jnp.dot(xn, w1b[:, cols128(i, n)], preferred_element_type=F32)
            hid[i, :, sl] = jax.nn.gelu(y + hid[i, :, sl], approximate=True)
            return c

        def g_piece(i, n, c):
            sl = slice(n * 128, (n + 1) * 128)
            return c + lax.dot_general(hid[i, :, sl].astype(BF16), w2b[:, cols128(i, n)],
                                       NT, preferred_element_type=F32)

        def k_piece(i, j, c):
            phase = i // NG
            s = lax.dot_general(qs[phase * 8 + j // 2].astype(BF16), kb[i, j], NT,
                                preferred_element_type=F32) * (DH ** -0.5)
            sc[i, j] = s
            mx[phase, j] = jnp.maximum(mx[phase, j], s)
            return c

        def v_piece(i, j, c):
            phase = i // NG
            p = jnp.exp(sc[i, j] - mx[phase, j])
            den[phase, j] += p
            acc[phase, j] += jnp.dot(p.astype(BF16), vb[i, j], preferred_element_type=F32)
            return c

        def wo_piece(i, n, c):
            sl = slice(n * 128, (n + 1) * 128)
            return c + lax.dot_general(att[i, :, sl].astype(BF16), wob[i, :, sl],
                                       NT, preferred_element_type=F32)

        pieces = {"q": (q_piece, 2), "h": (h_piece, 4), "g": (g_piece, 4),
                  "k": (k_piece, 16), "v": (v_piece, 16), "wo": (wo_piece, 4)}

        def step(kind, math, i, next_kind, next_i, slot, carry):
            for c in copies(kind, i, slot):
                c.wait()
            cps = copies(next_kind, next_i, slot) if next_kind else []
            todo = [(pieces[m][0], n) for m in math for n in range(pieces[m][1])]
            done = 0
            for u, (fn, n) in enumerate(todo):
                upto = (len(cps) * (u + 1)) // len(todo)
                start(cps, done, upto)
                done = upto
                carry = fn(i, n, carry)
            start(cps, done, len(cps))
            return carry

        carry = jnp.zeros((8, D), F32)
        gate = None
        prev = None
        for run in runs:
            (kind, i0), (next_kind, n0), t0 = run[0]
            math = math_for(kind, i0)
            if math != prev:
                if prev == ("g", "k"):
                    z = carry + b2b[...].astype(F32).reshape(1, D)
                    gate = z * jax.nn.sigmoid(z)
                    carry = jnp.zeros((8, D), F32)
                if prev == ("k",):
                    for p in range(NP):
                        for j in range(16):
                            mx[p, j] = jnp.broadcast_to(
                                jnp.max(mx[p, j], axis=-1, keepdims=True), (8, DH))
                if prev == ("v",):
                    for h in range(HKV):
                        p, j = h // 8, (h % 8) * 2
                        o = [acc[p, j + b] / jnp.sum(den[p, j + b], axis=-1, keepdims=True)
                             for b in range(2)]
                        o = jnp.where(first_batch, o[0], o[1])
                        c0 = (h % 2) * 256
                        att[h // 2, :, c0:c0 + 128] = jnp.where(first_head, o, 0.0)
                        att[h // 2, :, c0 + 128:c0 + 256] = jnp.where(first_head, 0.0, o)
                prev = math
            if len(run) == 1:
                carry = step(kind, math, i0, next_kind, n0, t0 % LOOKAHEAD, carry)
                continue

            def body(u, c, kind=kind, math=math, i0=i0, next_kind=next_kind, n0=n0, t0=t0):
                return step(kind, math, i0 + u, next_kind, (n0 + u) if next_kind else None,
                            lax.rem(t0 + u, LOOKAHEAD), c)

            if "g" in math or "wo" in math:
                carry = lax.fori_loop(0, len(run), body, carry)
            else:
                lax.fori_loop(0, len(run), body, 0)

        s8 = carry + pltpu.roll(carry, 6, 0)
        o_ref[...] = (x8 + s8 * gate)[0:2].astype(o_ref.dtype)

    scratch = [
        pltpu.VMEM((NP * NG, 16, GR, DH), BF16),
        pltpu.VMEM((NP * NG, 16, GR, DH), BF16),
        pltpu.VMEM((D, FQ), BF16),
        pltpu.VMEM((NQ, D, CB), BF16),
        pltpu.VMEM((D, FF), BF16),
        pltpu.VMEM((D, FF), BF16),
        pltpu.VMEM((2, D), BF16),
        pltpu.VMEM((FF,), BF16),
        pltpu.VMEM((D,), BF16),
        pltpu.VMEM((HKV, 8, DH), F32),
        pltpu.VMEM((NF, 8, CB), F32),
        pltpu.VMEM((NQ, 8, CB), F32),
        pltpu.VMEM((NP * NG, 16, 8, GR), F32),
        pltpu.VMEM((NP, 16, 8, DH), F32),
        pltpu.VMEM((NP, 16, 8, DH), F32),
        pltpu.VMEM((NP, 16, 8, DH), F32),
        pltpu.SemaphoreType.DMA((LOOKAHEAD,)),
        pltpu.SemaphoreType.DMA((3,)),
    ]
    return kernel, scratch


@jax.jit
def pallas_recurrent_scan__sliding_block_cached__dense_activation_gelu__decode_kernel(
    A_x: jax.Array,
    A_k_cache: jax.Array,
    A_v_cache: jax.Array,
    A_wq: jax.Array,
    A_wo: jax.Array,
    B_x: jax.Array,
    B_w1: jax.Array,
    B_b1: jax.Array,
    B_w2: jax.Array,
    B_b2: jax.Array,
):
    del B_x
    B, Sq, D = A_x.shape
    _, HKV, SK, dh = A_k_cache.shape
    W = min(4096, max(256, SK // 4))
    assert (B, Sq, dh) == (2, 1, DH) and GR == DH and A_wq.shape[1] == 2 * HKV * DH
    kernel, scratch = _make_kernel(D, HKV, SK, W, A_wq.shape[1], B_w1.shape[1])
    out = pl.pallas_call(
        kernel,
        out_shape=jax.ShapeDtypeStruct((B, D), A_x.dtype),
        in_specs=[pl.BlockSpec(memory_space=pltpu.HBM)] * 9,
        scratch_shapes=scratch,
        compiler_params=pltpu.CompilerParams(vmem_limit_bytes=110 * 2**20),
    )(A_x.reshape(B, D), A_k_cache, A_v_cache, A_wq, A_wo.T, B_w1, B_b1, B_w2.T, B_b2)
    return out.reshape(B, Sq, D)
```
